```python
import os as _os
_os.environ.setdefault('JAX_PLATFORMS', 'cpu')
import jax
import jax.numpy as jnp

def _softmax(x, axis=-1):
    return jax.nn.softmax(x, axis=axis)

def _gelu(x):
    return jax.nn.gelu(x, approximate=True)

def _silu(x):
    return jax.nn.silu(x)

def _sigmoid(x):
    return jax.nn.sigmoid(x)

def _layernorm(x, axis=-1, eps=1e-05):
    m = jnp.mean(x, axis=axis, keepdims=True)
    v = jnp.var(x, axis=axis, keepdims=True)
    return (x - m) / jnp.sqrt(v + eps)

def _scatter_add(tgt, idx, src, axis=0):
    return tgt.at[idx].add(src)

def _segment_sum(src, seg, n):
    return jax.ops.segment_sum(src, seg, n)

class _Rng:

    def __init__(self, key):
        self._k = key

    def _next(self):
        self._k, sub = jax.random.split(self._k)
        return sub

    def normal(self, shape):
        return jax.random.normal(self._next(), shape, dtype=jnp.bfloat16)

    def randint(self, lo, hi, shape):
        return jax.random.randint(self._next(), shape, lo, hi, dtype=jnp.int32)

    def uniform(self, shape, lo=0.0, hi=1.0):
        return jax.random.uniform(self._next(), shape, jnp.bfloat16, lo, hi)

    def permutation(self, n):
        return jax.random.permutation(self._next(), n)
kernel_name = 'standalone__conformer_conv_module__speech'

def setup_inputs():
    _rng = _Rng(jax.random.key(int.from_bytes(__import__("os").urandom(4), "little")))
    _w = lambda a: (lambda t: t.astype(jnp.bfloat16) if jnp.issubdtype(t.dtype, jnp.floating) else t)(jnp.asarray(a))
    B, T, D, K = (2, 16000, 256, 5)
    return {'x': _w((lambda *s: _rng.normal(s) * 0.2)(B, T, D)), 'w_pw1': _w((lambda *s: _rng.normal(s) * 0.2)(D, 2 * D)), 'dw': _w((lambda *s: _rng.normal(s) * 0.05)(K, D)), 'w_pw2': _w((lambda *s: _rng.normal(s) * 0.05)(D, D))}

def reference(x, w_pw1, dw, w_pw2):
    B, T, D = x.shape
    K = dw.shape[0]
    h = x @ w_pw1
    a, b = (h[..., :D].copy(), h[..., D:].copy())
    h = a * _sigmoid(b)
    pad = K // 2
    hp = jnp.pad(h, ((0, 0), (pad, pad), (0, 0)))
    out = jnp.zeros_like(h)
    for i in range(K):
        out = out + hp[:, i:i + T, :] * dw[i][None, None, :]
    return _silu(out) @ w_pw2
```

```python
import functools
import jax
import jax.numpy as jnp
import jax.experimental.pallas as pl
import jax.experimental.pallas.tpu as pltpu

TT = 2000
R = 400
H = 16
G = 8
L = 128

def _glu2(xs, w1_ref, D):
    hh = jnp.dot(xs, w1_ref[...], preferred_element_type=jnp.float32)
    a = hh[:, :D]; b = hh[:, D:]
    return a * (1.0 + jnp.tanh(0.5 * b))

def _kernel(x_ref, xh_ref, w1_ref, dw_ref, w2_ref, o_ref, *hbufs, nT, D, K):
    t = pl.program_id(1)
    pad = K // 2
    nC = TT // R
    nL = D // L
    zero = jnp.minimum(t, 0)

    def store_h(buf, start, h):
        for j in range(nL):
            buf[j, pl.ds(start, h.shape[0]), :] = h[:, j * L:(j + 1) * L]

    @pl.when(t == 0)
    def _():
        store_h(hbufs[0], 0, jnp.zeros((G, D), jnp.float32))
        store_h(hbufs[0], G, _glu2(x_ref[0, pl.ds(0, H), :], w1_ref, D))

    dwf = dw_ref[...].astype(jnp.float32) * 0.25

    def A(c):
        if c < nC - 1:
            xs = x_ref[0, pl.ds(H + c * R, R), :]
            h = _glu2(xs, w1_ref, D)
        else:
            xs = jnp.concatenate([x_ref[0, pl.ds(H + c * R, R - H), :], xh_ref[0]], axis=0)
            h = _glu2(xs, w1_ref, D)
            row = jax.lax.broadcasted_iota(jnp.int32, (R, D), 0)
            valid = jnp.logical_or(row < R - H, t < nT - 1)
            h = jnp.where(valid, h, 0.0)
        store_h(hbufs[c], G + H, h[:R - H + G])
        store_h(hbufs[(c + 1) % nC], 0, h[R - H - G:])

    def Bc(c):
        ss = []
        for j in range(nL):
            acc = None
            for k in range(K):
                tk = hbufs[c][j, pl.ds(zero + (G - pad + k), R), :] * dwf[k:k + 1, j * L:(j + 1) * L]
                acc = tk if acc is None else acc + tk
            ss.append(acc * (1.0 + jnp.tanh(acc)))
        s = jnp.concatenate(ss, axis=1)
        o = jnp.dot(s.astype(jnp.bfloat16), w2_ref[...], preferred_element_type=jnp.float32)
        o_ref[0, pl.ds(c * R, R), :] = o.astype(o_ref.dtype)

    A(0)
    for c in range(nC):
        if c + 1 < nC:
            A(c + 1)
        Bc(c)


@jax.jit
def pallas_standalone__conformer_conv_module__speech_kernel(x, w_pw1, dw, w_pw2):
    B, T, D = x.shape
    K = dw.shape[0]
    nT = T // TT
    kern = functools.partial(_kernel, nT=nT, D=D, K=K)
    nH = T // H
    return pl.pallas_call(
        kern,
        grid=(B, nT),
        in_specs=[
            pl.BlockSpec((1, TT, D), lambda b, t: (b, t, 0)),
            pl.BlockSpec((1, H, D), lambda b, t: (b, jnp.minimum((t + 1) * (TT // H), nH - 1), 0)),
            pl.BlockSpec((D, 2 * D), lambda b, t: (0, 0)),
            pl.BlockSpec((K, D), lambda b, t: (0, 0)),
            pl.BlockSpec((D, D), lambda b, t: (0, 0)),
        ],
        out_specs=pl.BlockSpec((1, TT, D), lambda b, t: (b, t, 0)),
        out_shape=jax.ShapeDtypeStruct((B, T, D), x.dtype),
        scratch_shapes=[pltpu.VMEM((D // L, R + 2 * G, L), jnp.float32) for _ in range(TT // R)],
        compiler_params=pltpu.CompilerParams(
            dimension_semantics=("arbitrary", "arbitrary"),
            vmem_limit_bytes=64 * 1024 * 1024,
        ),
    )(x, x, w_pw1, dw, w_pw2)
```

```python
import functools
import jax
import jax.numpy as jnp
import jax.experimental.pallas as pl
import jax.experimental.pallas.tpu as pltpu

R = 400
S = 10
P = 3
M = 7
HEAD_WAITS = (1, 2)
TAIL_FLUSH = (2, 4, 5)
EARLY = 2
WIN0_AT = 0
H = 16
G = 8
L = 128

def _kernel(x_hbm, w1_hbm, dw_hbm, w2_hbm, o_hbm,
            xbuf, xh, obuf, w1_ref, dw_ref, w2_ref, *rest, N, T, D, K):
    hbufs = rest[:S]
    xsem, osem, wsem, psem, tsem = rest[S:]
    TT = S * R
    nchunks = N // R
    Q = nchunks - 1 - P - M * S
    assert Q >= 1 and T % R == 0 and M >= 2 and Q + 1 <= S and P <= S
    cpb = T // R
    pad = K // 2
    nL = D // L
    g0 = P + 1
    zero = jnp.minimum(pl.program_id(0), 0)

    def x_copy(i, slot, rows):
        return pltpu.make_async_copy(
            x_hbm.at[pl.ds((g0 + i * S) * R + H, rows), :], xbuf.at[slot, pl.ds(0, rows), :], xsem.at[slot])

    def o_copy(row0, slot, rows):
        return pltpu.make_async_copy(
            obuf.at[slot, pl.ds(0, rows), :], o_hbm.at[pl.ds(row0, rows), :], osem.at[slot])

    bounds = [0] + [c * R + H for c in HEAD_WAITS] + [(P + 1) * R + H]
    pieces = [pltpu.make_async_copy(x_hbm.at[pl.ds(bounds[k], bounds[k + 1] - bounds[k]), :],
                                    xh.at[pl.ds(bounds[k], bounds[k + 1] - bounds[k]), :], psem.at[k])
              for k in range(len(bounds) - 1)]
    w1_cp = pltpu.make_async_copy(w1_hbm, w1_ref, wsem.at[0])
    dw_cp = pltpu.make_async_copy(dw_hbm, dw_ref, wsem.at[1])
    w2_cp = pltpu.make_async_copy(w2_hbm, w2_ref, wsem.at[2])

    w1_cp.start(); pieces[0].start()
    if EARLY >= 1:
        pieces[1].start()
    if EARLY >= 2:
        for pc in pieces[2:]:
            pc.start()

    def glu2(xs):
        hh = jnp.dot(xs, w1_ref[...], preferred_element_type=jnp.float32)
        a = hh[:, :D]; b = hh[:, D:]
        return a * (1.0 + jnp.tanh(0.5 * b))

    def store_h(buf, start, h):
        for j in range(nL):
            buf[j, pl.ds(start, h.shape[0]), :] = h[:, j * L:(j + 1) * L]

    def A(xs, bc, edge):
        h = glu2(xs)
        store_h(hbufs[bc], G + H, h[:R - H])
        tail = h[R - H - G:]
        if edge is None:
            store_h(hbufs[bc], G + R, tail[G:2 * G])
            store_h(hbufs[(bc + 1) % S], 0, tail)
        else:
            store_h(hbufs[bc], G + R, jnp.where(edge, 0.0, tail[G:2 * G]))
            store_h(hbufs[(bc + 1) % S], 0, jnp.where(edge, 0.0, tail[:G]))
            store_h(hbufs[(bc + 1) % S], G, tail[G:])

    def static_edge(g):
        return True if (g + 1) % cpb == 0 else None

    def Bc(c, oslot, off):
        dwf = dw_ref[...].astype(jnp.float32) * 0.25
        ss = []
        for j in range(nL):
            acc = None
            for k in range(K):
                tk = hbufs[c][j, pl.ds(zero + (G - pad + k), R), :] * dwf[k:k + 1, j * L:(j + 1) * L]
                acc = tk if acc is None else acc + tk
            ss.append(acc * (1.0 + jnp.tanh(acc)))
        s = jnp.concatenate(ss, axis=1)
        o = jnp.dot(s.astype(jnp.bfloat16), w2_ref[...], preferred_element_type=jnp.float32)
        obuf[oslot, pl.ds(off, R), :] = o.astype(obuf.dtype)

    w1_cp.wait(); pieces[0].wait()
    if EARLY < 1:
        pieces[1].start()
    dw_cp.start(); w2_cp.start()
    if EARLY < 2:
        for pc in pieces[2:]:
            pc.start()
    if WIN0_AT == 0:
        x_copy(0, 0, TT).start()
    h0 = glu2(xh[pl.ds(0, R + H), :])
    store_h(hbufs[0], 0, jnp.zeros((G, D), jnp.float32))
    store_h(hbufs[0], G, h0[:R + G])
    store_h(hbufs[1], 0, h0[R - G:])
    for g in range(1, P + 1):
        if g in HEAD_WAITS:
            pieces[HEAD_WAITS.index(g) + 1].wait()
        if g == 1:
            dw_cp.wait(); w2_cp.wait()
        if g == WIN0_AT:
            x_copy(0, 0, TT).start()
        A(xh[pl.ds(g * R + H, R), :], g % S, static_edge(g))
        Bc((g - 1) % S, 1, (g - 1) * R)
    o_copy(0, 1, P * R).start()

    TAILX = Q * R - H
    def body(i, carry):
        slot = i % 2
        x_copy(i, slot, TT).wait()

        @pl.when(i + 1 < M)
        def _():
            x_copy(i + 1, 1 - slot, TT).start()

        @pl.when(i + 1 == M)
        def _():
            x_copy(i + 1, 1 - slot, TAILX).start()

        @pl.when(i == 1)
        def _():
            o_copy(0, 1, P * R).wait()

        @pl.when(i >= 2)
        def _():
            o_copy(0, slot, TT).wait()

        for c in range(S):
            g = g0 + i * S + c
            A(xbuf[slot, pl.ds(c * R, R), :], (g0 + c) % S, ((g + 1) % cpb) == 0)
            Bc((g0 + c - 1) % S, slot, c * R)
        o_copy((P + i * S) * R, slot, TT).start()
        return carry

    jax.lax.fori_loop(0, M, body, 0)

    ts = M % 2
    x_copy(M, ts, TAILX).wait()
    o_copy(0, ts, TT).wait()
    gt = g0 + M * S
    flushed = 0
    tail_cps = []
    for q in range(Q + 1):
        g = gt + q
        if q < Q:
            A(xbuf[ts, pl.ds(q * R, R), :], g % S, static_edge(g))
        Bc((g - 1) % S, ts, q * R)
        if q in TAIL_FLUSH or q == Q:
            cp = pltpu.make_async_copy(obuf.at[ts, pl.ds(flushed * R, (q + 1 - flushed) * R), :],
                                       o_hbm.at[pl.ds((gt - 1 + flushed) * R, (q + 1 - flushed) * R), :],
                                       tsem.at[len(tail_cps)])
            cp.start(); tail_cps.append(cp); flushed = q + 1
    o_copy(0, 1 - ts, TT).wait()
    for cp in tail_cps:
        cp.wait()


@jax.jit
def pallas_standalone__conformer_conv_module__speech_kernel(x, w_pw1, dw, w_pw2):
    B, T, D = x.shape
    K = dw.shape[0]
    N = B * T
    TT = S * R
    kern = functools.partial(_kernel, N=N, T=T, D=D, K=K)
    any_spec = pl.BlockSpec(memory_space=pl.ANY)
    out = pl.pallas_call(
        kern,
        grid=(1,),
        in_specs=[any_spec] * 4,
        out_specs=any_spec,
        out_shape=jax.ShapeDtypeStruct((N, D), x.dtype),
        scratch_shapes=[
            pltpu.VMEM((2, TT, D), x.dtype),
            pltpu.VMEM(((P + 1) * R + H, D), x.dtype),
            pltpu.VMEM((2, TT, D), x.dtype),
            pltpu.VMEM((D, 2 * D), w_pw1.dtype),
            pltpu.VMEM((K, D), dw.dtype),
            pltpu.VMEM((D, D), w_pw2.dtype),
        ] + [pltpu.VMEM((D // L, R + 2 * G, L), jnp.float32) for _ in range(S)] + [
            pltpu.SemaphoreType.DMA((2,)),
            pltpu.SemaphoreType.DMA((2,)),
            pltpu.SemaphoreType.DMA((3,)),
            pltpu.SemaphoreType.DMA((len(HEAD_WAITS) + 1,)),
            pltpu.SemaphoreType.DMA((len(TAIL_FLUSH) + 1,)),
        ],
        compiler_params=pltpu.CompilerParams(
            dimension_semantics=("arbitrary",),
            vmem_limit_bytes=64 * 1024 * 1024,
        ),
    )(x.reshape(N, D), w_pw1, dw, w_pw2)
    return out.reshape(B, T, D)
```

```python
import functools

import jax
import jax.numpy as jnp
import jax.experimental.pallas as pl
import jax.experimental.pallas.tpu as pltpu

R = 400
S = 10
P = 3
M = 7
HEAD_WAITS = (1, 2)
TAIL_FLUSH = (2, 4, 5)
H = 16
G = 8
L = 128


def _kernel(x_hbm, w1_hbm, dw_hbm, w2_hbm, o_hbm,
            xbuf, xh, obuf, w1_ref, dw_ref, w2_ref, *rest, N, T, D, K):
    hbufs = rest[:S]
    xsem, osem, wsem, psem, tsem = rest[S:]
    TT = S * R
    nchunks = N // R
    Q = nchunks - 1 - P - M * S
    pad = K // 2
    assert Q >= 1 and Q + 1 <= S and P <= S and M >= 2
    assert T % R == 0 and N == nchunks * R and pad <= G and D % L == 0
    cpb = T // R
    nL = D // L
    g0 = P + 1
    tail_rows = Q * R - H
    zero = jnp.minimum(pl.program_id(0), 0)

    def x_copy(i, slot, rows):
        return pltpu.make_async_copy(
            x_hbm.at[pl.ds((g0 + i * S) * R + H, rows), :],
            xbuf.at[slot, pl.ds(0, rows), :], xsem.at[slot])

    def o_copy(row0, slot, rows):
        return pltpu.make_async_copy(
            obuf.at[slot, pl.ds(0, rows), :],
            o_hbm.at[pl.ds(row0, rows), :], osem.at[slot])

    bounds = [0] + [c * R + H for c in HEAD_WAITS] + [(P + 1) * R + H]
    pieces = [
        pltpu.make_async_copy(
            x_hbm.at[pl.ds(bounds[k], bounds[k + 1] - bounds[k]), :],
            xh.at[pl.ds(bounds[k], bounds[k + 1] - bounds[k]), :], psem.at[k])
        for k in range(len(bounds) - 1)]
    w1_cp = pltpu.make_async_copy(w1_hbm, w1_ref, wsem.at[0])
    dw_cp = pltpu.make_async_copy(dw_hbm, dw_ref, wsem.at[1])
    w2_cp = pltpu.make_async_copy(w2_hbm, w2_ref, wsem.at[2])

    w1_cp.start()
    for pc in pieces:
        pc.start()

    def glu2(xs):
        hh = jnp.dot(xs, w1_ref[...], preferred_element_type=jnp.float32)
        a = hh[:, :D]
        b = hh[:, D:]
        return a * (1.0 + jnp.tanh(0.5 * b))

    def store_h(buf, start, h):
        for j in range(nL):
            buf[j, pl.ds(start, h.shape[0]), :] = h[:, j * L:(j + 1) * L]

    def stage_a(xs, bc, edge):
        h = glu2(xs)
        store_h(hbufs[bc], G + H, h[:R - H])
        tail = h[R - H - G:]
        nxt = hbufs[(bc + 1) % S]
        if edge is None:
            store_h(hbufs[bc], G + R, tail[G:2 * G])
            store_h(nxt, 0, tail)
        else:
            store_h(hbufs[bc], G + R, jnp.where(edge, 0.0, tail[G:2 * G]))
            store_h(nxt, 0, jnp.where(edge, 0.0, tail[:G]))
            store_h(nxt, G, tail[G:])

    def static_edge(g):
        return True if (g + 1) % cpb == 0 else None

    def stage_b(bc, oslot, off):
        dwf = dw_ref[...].astype(jnp.float32) * 0.25
        ss = []
        for j in range(nL):
            acc = None
            for k in range(K):
                tk = (hbufs[bc][j, pl.ds(zero + (G - pad + k), R), :]
                      * dwf[k:k + 1, j * L:(j + 1) * L])
                acc = tk if acc is None else acc + tk
            ss.append(acc * (1.0 + jnp.tanh(acc)))
        s = jnp.concatenate(ss, axis=1)
        o = jnp.dot(s.astype(w2_ref.dtype), w2_ref[...], preferred_element_type=jnp.float32)
        obuf[oslot, pl.ds(off, R), :] = o.astype(obuf.dtype)

    w1_cp.wait()
    pieces[0].wait()
    dw_cp.start()
    w2_cp.start()
    x_copy(0, 0, TT).start()
    h0 = glu2(xh[pl.ds(0, R + H), :])
    store_h(hbufs[0], 0, jnp.zeros((G, D), jnp.float32))
    store_h(hbufs[0], G, h0[:R + G])
    store_h(hbufs[1], 0, h0[R - G:])
    for g in range(1, P + 1):
        if g in HEAD_WAITS:
            pieces[HEAD_WAITS.index(g) + 1].wait()
        if g == 1:
            dw_cp.wait()
            w2_cp.wait()
        stage_a(xh[pl.ds(g * R + H, R), :], g % S, static_edge(g))
        stage_b((g - 1) % S, 1, (g - 1) * R)
    o_copy(0, 1, P * R).start()

    def body(i, carry):
        slot = jax.lax.bitwise_and(i, 1)
        x_copy(i, slot, TT).wait()

        @pl.when(i + 1 < M)
        def _():
            x_copy(i + 1, 1 - slot, TT).start()

        @pl.when(i + 1 == M)
        def _():
            x_copy(i + 1, 1 - slot, tail_rows).start()

        @pl.when(i == 1)
        def _():
            o_copy(0, 1, P * R).wait()

        @pl.when(i >= 2)
        def _():
            o_copy(0, slot, TT).wait()

        for c in range(S):
            g = g0 + i * S + c
            stage_a(xbuf[slot, pl.ds(c * R, R), :], (g0 + c) % S, ((g + 1) % cpb) == 0)
            stage_b((g0 + c - 1) % S, slot, c * R)
        o_copy((P + i * S) * R, slot, TT).start()
        return carry

    jax.lax.fori_loop(0, M, body, 0)

    ts = M % 2
    x_copy(M, ts, tail_rows).wait()
    o_copy(0, ts, TT).wait()
    gt = g0 + M * S
    flushed = 0
    tail_cps = []
    for q in range(Q + 1):
        g = gt + q
        if q < Q:
            stage_a(xbuf[ts, pl.ds(q * R, R), :], g % S, static_edge(g))
        stage_b((g - 1) % S, ts, q * R)
        if q in TAIL_FLUSH or q == Q:
            rows = (q + 1 - flushed) * R
            cp = pltpu.make_async_copy(
                obuf.at[ts, pl.ds(flushed * R, rows), :],
                o_hbm.at[pl.ds((gt - 1 + flushed) * R, rows), :], tsem.at[len(tail_cps)])
            cp.start()
            tail_cps.append(cp)
            flushed = q + 1
    o_copy(0, 1 - ts, TT).wait()
    for cp in tail_cps:
        cp.wait()


@jax.jit
def pallas_standalone__conformer_conv_module__speech_kernel(
    x: jax.Array,
    w_pw1: jax.Array,
    dw: jax.Array,
    w_pw2: jax.Array,
):
    B, T, D = x.shape
    K = dw.shape[0]
    N = B * T
    TT = S * R
    any_spec = pl.BlockSpec(memory_space=pl.ANY)
    out = pl.pallas_call(
        functools.partial(_kernel, N=N, T=T, D=D, K=K),
        grid=(1,),
        in_specs=[any_spec] * 4,
        out_specs=any_spec,
        out_shape=jax.ShapeDtypeStruct((N, D), x.dtype),
        scratch_shapes=[
            pltpu.VMEM((2, TT, D), x.dtype),
            pltpu.VMEM(((P + 1) * R + H, D), x.dtype),
            pltpu.VMEM((2, TT, D), x.dtype),
            pltpu.VMEM((D, 2 * D), w_pw1.dtype),
            pltpu.VMEM((K, D), dw.dtype),
            pltpu.VMEM((D, D), w_pw2.dtype),
        ] + [pltpu.VMEM((D // L, R + 2 * G, L), jnp.float32) for _ in range(S)] + [
            pltpu.SemaphoreType.DMA((2,)),
            pltpu.SemaphoreType.DMA((2,)),
            pltpu.SemaphoreType.DMA((3,)),
            pltpu.SemaphoreType.DMA((len(HEAD_WAITS) + 1,)),
            pltpu.SemaphoreType.DMA((len(TAIL_FLUSH) + 1,)),
        ],
        compiler_params=pltpu.CompilerParams(
            dimension_semantics=("arbitrary",),
            vmem_limit_bytes=64 * 1024 * 1024,
            disable_bounds_checks=True,
        ),
    )(x.reshape(N, D), w_pw1, dw, w_pw2)
    return out.reshape(B, T, D)
```
